```python
import os as _os
_os.environ.setdefault("JAX_PLATFORMS", "cpu")
import jax
import jax.numpy as jnp

def _softmax(x, axis=-1):
    return jax.nn.softmax(x, axis=axis)
def _gelu(x):
    return jax.nn.gelu(x, approximate=True)
def _silu(x):
    return jax.nn.silu(x)
def _sigmoid(x):
    return jax.nn.sigmoid(x)
def _layernorm(x, axis=-1, eps=1e-5):
    m = jnp.mean(x, axis=axis, keepdims=True)
    v = jnp.var(x, axis=axis, keepdims=True)
    return (x - m) / jnp.sqrt(v + eps)
def _scatter_add(tgt, idx, src, axis=0):
    return tgt.at[idx].add(src)
def _segment_sum(src, seg, n):
    return jax.ops.segment_sum(src, seg, n)
class _Rng:
    def __init__(self, key):
        self._k = key
    def _next(self):
        self._k, sub = jax.random.split(self._k)
        return sub
    def normal(self, shape):
        return jax.random.normal(self._next(), shape, dtype=jnp.bfloat16)
    def randint(self, lo, hi, shape):
        return jax.random.randint(self._next(), shape, lo, hi, dtype=jnp.int32)
    def uniform(self, shape, lo=0.0, hi=1.0):
        return jax.random.uniform(self._next(), shape, jnp.bfloat16, lo, hi)
    def permutation(self, n):
        return jax.random.permutation(self._next(), n)


kernel_name = 'standalone__gqa_block_cached__near_ridge'

def setup_inputs():
    _rng = _Rng(jax.random.key(int.from_bytes(__import__("os").urandom(4), "little")))
    _w = (lambda a: (lambda t: t.astype(jnp.bfloat16) if jnp.issubdtype(t.dtype, jnp.floating) else t)(jnp.asarray(a)))
    B, Sq, D = 8, 96, 640
    Hq, Hkv, Sk, Dh = 32, 32, 512, 128
    assert Hq % Hkv == 0, (Hq, Hkv)
    return {
        "x": _w((lambda *s: _rng.normal(s) * 0.2)(B, Sq, D)),
        "k_cache": _w((lambda *s: _rng.normal(s) * 3.2)(B, Hkv, Sk, Dh)),
        "v_cache": _w((lambda *s: _rng.normal(s) * 0.05)(B, Hkv, Sk, Dh)),
        "wq": _w((lambda *s: _rng.normal(s) * 0.2)(D, Hq * Dh) * (D ** -0.5)),
        "wo": _w((lambda *s: _rng.normal(s) * 0.05)(Hq * Dh, D) * ((Hq * Dh) ** -0.5)),
    }

def reference(x, k_cache, v_cache, wq, wo):
    B, Sq, D = x.shape
    Hq, Dh = 32, 128
    Hkv = k_cache.shape[1]
    rep = Hq // Hkv
    q = (lambda x, *d: x.transpose(*d))((x @ wq).reshape(B, Sq, Hq, Dh), 0, 2, 1, 3)
    k = jnp.repeat(k_cache, rep, axis=1)
    v = jnp.repeat(v_cache, rep, axis=1)
    scores = jnp.einsum("bhqd,bhkd->bhqk", q, k) * (Dh ** -0.5)
    p = _softmax(scores, axis=-1)
    o = jnp.einsum("bhqk,bhkd->bhqd", p, v)
    return (lambda x, *d: x.transpose(*d))(o, 0, 2, 1, 3).reshape(B, Sq, Hq * Dh) @ wo
```

```python
import functools

import jax
import jax.numpy as jnp
from jax import lax
import jax.experimental.pallas as pl
import jax.experimental.pallas.tpu as pltpu


def _kernel(x_ref, k_ref, v_ref, wq_ref, wo_ref, o_ref, acc_ref, q_ref, oh_ref,
            *, B, Sq, scale):
    h = pl.program_id(0)
    nh = pl.num_programs(0)

    q = jnp.dot(x_ref[...], wq_ref[...], preferred_element_type=jnp.float32)
    q_ref[...] = q.astype(q_ref.dtype)

    for b in range(B):
        qb = q_ref[b * Sq:(b + 1) * Sq, :]
        k = k_ref[b, 0]
        s = lax.dot_general(qb, k, (((1,), (1,)), ((), ())),
                            preferred_element_type=jnp.float32) * scale
        m = jnp.max(s, axis=-1, keepdims=True)
        p = jnp.exp(s - m)
        l = jnp.sum(p, axis=-1, keepdims=True)
        o = jnp.dot(p.astype(jnp.bfloat16), v_ref[b, 0],
                    preferred_element_type=jnp.float32)
        o = o / l
        oh_ref[b * Sq:(b + 1) * Sq, :] = o.astype(oh_ref.dtype)

    contrib = jnp.dot(oh_ref[...], wo_ref[...], preferred_element_type=jnp.float32)

    @pl.when(h == 0)
    def _():
        acc_ref[...] = contrib

    @pl.when(h > 0)
    def _():
        acc_ref[...] += contrib

    @pl.when(h == nh - 1)
    def _():
        o_ref[...] = acc_ref[...].astype(o_ref.dtype)


@jax.jit
def pallas_standalone__gqa_block_cached__near_ridge_kernel(
    x: jax.Array,
    k_cache: jax.Array,
    v_cache: jax.Array,
    wq: jax.Array,
    wo: jax.Array,
):
    B, Sq, D = x.shape
    Hq, Dh = 32, 128
    Hkv, Sk = k_cache.shape[1], k_cache.shape[2]
    rep = Hq // Hkv
    M = B * Sq
    x2 = x.reshape(M, D)

    kern = functools.partial(_kernel, B=B, Sq=Sq, scale=float(Dh) ** -0.5)
    out = pl.pallas_call(
        kern,
        grid=(Hq,),
        in_specs=[
            pl.BlockSpec((M, D), lambda h: (0, 0)),
            pl.BlockSpec((B, 1, Sk, Dh), lambda h: (0, h // rep, 0, 0)),
            pl.BlockSpec((B, 1, Sk, Dh), lambda h: (0, h // rep, 0, 0)),
            pl.BlockSpec((D, Dh), lambda h: (0, h)),
            pl.BlockSpec((Dh, D), lambda h: (h, 0)),
        ],
        out_specs=pl.BlockSpec((M, D), lambda h: (0, 0)),
        out_shape=jax.ShapeDtypeStruct((M, D), x.dtype),
        scratch_shapes=[
            pltpu.VMEM((M, D), jnp.float32),
            pltpu.VMEM((M, Dh), jnp.bfloat16),
            pltpu.VMEM((M, Dh), jnp.bfloat16),
        ],
        compiler_params=pltpu.CompilerParams(
            dimension_semantics=("arbitrary",),
            vmem_limit_bytes=64 * 1024 * 1024,
        ),
    )(x2, k_cache, v_cache, wq, wo)
    return out.reshape(B, Sq, D)
```

```python
import functools

import jax
import jax.numpy as jnp
from jax import lax
import jax.experimental.pallas as pl
import jax.experimental.pallas.tpu as pltpu

_NB = 4
_NCH = 2


def _kernel(x_hbm, k_hbm, v_hbm, wq_hbm, wo_hbm, o_hbm,
            x_buf, k_buf, v_buf, wq_buf, wo_buf,
            acc_ref, q_ref, s_ref, p_ref, l_ref, oh_ref, ostage,
            sems, sems_last, sem_x, sem_o,
            *, B, Sq, H, Dh, rep, scale, vch):
    NB, NCH = _NB, _NCH
    HB = B // NCH
    PD = NB - 2
    LSLOT = (H - 1) % NB

    def rows(b):
        return slice(b * Sq, (b + 1) * Sq)

    def wq_copy(h, slot):
        off = pl.multiple_of(h * Dh, Dh)
        return pltpu.make_async_copy(
            wq_hbm.at[:, pl.ds(off, Dh)], wq_buf.at[slot], sems.at[0, slot])

    def wo_copy(h, slot):
        off = pl.multiple_of(h * Dh, Dh)
        return pltpu.make_async_copy(
            wo_hbm.at[pl.ds(off, Dh), :], wo_buf.at[slot], sems.at[1, slot])

    def k_copy(h, slot, c):
        return pltpu.make_async_copy(
            k_hbm.at[pl.ds(c * HB, HB), h // rep],
            k_buf.at[slot, pl.ds(c * HB, HB)], sems.at[2 + c, slot])

    def v_copy(h, slot, c):
        return pltpu.make_async_copy(
            v_hbm.at[pl.ds(c * HB, HB), h // rep],
            v_buf.at[slot, pl.ds(c * HB, HB)], sems.at[2 + NCH + c, slot])

    def v_last_copy(i):
        b0, b1 = vch[i]
        return pltpu.make_async_copy(
            v_hbm.at[pl.ds(b0, b1 - b0), (H - 1) // rep],
            v_buf.at[LSLOT, pl.ds(b0, b1 - b0)], sems_last.at[i])

    def out_copy(b):
        return pltpu.make_async_copy(
            ostage.at[rows(b), :], o_hbm.at[rows(b), :], sem_o.at[b])

    def start_head(h, slot):
        for c in range(NCH):
            k_copy(h, slot, c).start()
            v_copy(h, slot, c).start()
            if c == 0:
                wo_copy(h, slot).start()

    def start_last():
        for c in range(NCH):
            k_copy(H - 1, LSLOT, c).start()
        wo_copy(H - 1, LSLOT).start()
        for i in range(len(vch)):
            v_last_copy(i).start()

    x_copy = pltpu.make_async_copy(x_hbm, x_buf, sem_x)
    x_copy.start()
    wq_copy(0, 0).start()
    wq_copy(1, 1).start()
    for i in range(PD):
        start_head(i, i)
        wq_copy(i + 2, (i + 2) % NB).start()

    acc_ref[...] = jnp.zeros_like(acc_ref)
    s_ref[rows(B - 1), :] = jnp.zeros((Sq, s_ref.shape[1]), s_ref.dtype)
    p_ref[rows(B - 2), :] = jnp.zeros((Sq, p_ref.shape[1]), p_ref.dtype)
    l_ref[rows(B - 2), :] = jnp.ones((Sq, 1), l_ref.dtype)
    oh_ref[rows(B - 3), :] = jnp.zeros((Sq, Dh), oh_ref.dtype)
    x_copy.wait()
    wq_copy(0, 0).wait()
    q_ref[0] = jnp.dot(x_buf[...], wq_buf[0],
                       preferred_element_type=jnp.float32).astype(q_ref.dtype)

    def qproj(b, qs, wslot):
        q_ref[qs, rows(b), :] = jnp.dot(
            x_buf[rows(b), :], wq_buf[wslot],
            preferred_element_type=jnp.float32).astype(q_ref.dtype)

    def qk(b, qs, slot):
        s_ref[rows(b), :] = lax.dot_general(
            q_ref[qs, rows(b), :], k_buf[slot, b], (((1,), (1,)), ((), ())),
            preferred_element_type=jnp.float32)

    def softmax(b):
        s = s_ref[rows(b), :]
        m = jnp.max(s, axis=-1, keepdims=True)
        p = jnp.exp((s - m) * scale)
        l_ref[rows(b), :] = jnp.sum(p, axis=-1, keepdims=True)
        p_ref[rows(b), :] = p.astype(p_ref.dtype)

    def pv(b, slot, flag=None):
        o = jnp.dot(p_ref[rows(b), :], v_buf[slot, b],
                    preferred_element_type=jnp.float32)
        o = o / l_ref[rows(b), :]
        if flag is not None:
            o = o * flag
        oh_ref[rows(b), :] = o.astype(oh_ref.dtype)

    def outp(b, slot, final=False):
        r = acc_ref[rows(b), :] + jnp.dot(
            oh_ref[rows(b), :], wo_buf[slot],
            preferred_element_type=jnp.float32)
        if final:
            ostage[rows(b), :] = r.astype(ostage.dtype)
            out_copy(b).start()
        else:
            acc_ref[rows(b), :] = r

    def body(h, carry):
        slot = h % NB
        pslot = jnp.maximum(h - 1, 0) % NB
        qs = h % 2
        flag = (h > 0).astype(jnp.float32)
        nxt = h + PD

        @pl.when(nxt < H - 1)
        def _():
            start_head(nxt, nxt % NB)

        @pl.when(nxt == H - 1)
        def _():
            start_last()

        @pl.when(nxt + 2 < H)
        def _():
            wq_copy(nxt + 2, (nxt + 2) % NB).start()

        wslot = (h + 1) % NB
        wq_copy(h + 1, wslot).wait()
        wo_copy(h, slot).wait()
        for t in range(B):
            if t % HB == 0:
                k_copy(h, slot, t // HB).wait()
                v_copy(h, slot, t // HB).wait()
            qk(t, qs, slot)
            softmax((t - 1) % B)
            if t >= 2:
                pv(t - 2, slot)
            else:
                pv(B + t - 2, pslot, flag)
            if t >= 3:
                outp(t - 3, slot)
            else:
                outp(B + t - 3, pslot)
            qproj(t, 1 - qs, wslot)
        return carry

    lax.fori_loop(0, H - 1, body, 0)

    qs = (H - 1) % 2
    pslot = (H - 2) % NB
    for t in range(B + 1):
        if t < B and t % HB == 0:
            k_copy(H - 1, LSLOT, t // HB).wait()
        if t < B:
            qk(t, qs, LSLOT)
        softmax((t - 1) % B)
        if t < 2:
            pv(B + t - 2, pslot)
        if t < 3:
            outp(B + t - 3, pslot)
    wo_copy(H - 1, LSLOT).wait()
    for i, (b0, b1) in enumerate(vch):
        v_last_copy(i).wait()
        for b in range(b0, b1):
            pv(b, LSLOT)
        for b in range(b0, b1):
            outp(b, LSLOT, final=True)
    for b in range(B):
        out_copy(b).wait()


@jax.jit
def pallas_standalone__gqa_block_cached__near_ridge_kernel(
    x: jax.Array,
    k_cache: jax.Array,
    v_cache: jax.Array,
    wq: jax.Array,
    wo: jax.Array,
):
    B, Sq, D = x.shape
    Hq, Dh = 32, 128
    Hkv, Sk = k_cache.shape[1], k_cache.shape[2]
    rep = Hq // Hkv
    M = B * Sq
    x2 = x.reshape(M, D)
    vch = ((0, B // 2), (B // 2, B - 1), (B - 1, B))

    kern = functools.partial(_kernel, B=B, Sq=Sq, H=Hq, Dh=Dh, rep=rep,
                             scale=float(Dh) ** -0.5, vch=vch)
    any_spec = pl.BlockSpec(memory_space=pl.ANY)
    out = pl.pallas_call(
        kern,
        in_specs=[any_spec] * 5,
        out_specs=any_spec,
        out_shape=jax.ShapeDtypeStruct((M, D), x.dtype),
        scratch_shapes=[
            pltpu.VMEM((M, D), x.dtype),
            pltpu.VMEM((_NB, B, Sk, Dh), k_cache.dtype),
            pltpu.VMEM((_NB, B, Sk, Dh), v_cache.dtype),
            pltpu.VMEM((_NB, D, Dh), wq.dtype),
            pltpu.VMEM((_NB, Dh, D), wo.dtype),
            pltpu.VMEM((M, D), jnp.float32),
            pltpu.VMEM((2, M, Dh), jnp.bfloat16),
            pltpu.VMEM((M, Sk), jnp.float32),
            pltpu.VMEM((M, Sk), jnp.bfloat16),
            pltpu.VMEM((M, 1), jnp.float32),
            pltpu.VMEM((M, Dh), jnp.bfloat16),
            pltpu.VMEM((M, D), x.dtype),
            pltpu.SemaphoreType.DMA((2 + 2 * _NCH, _NB)),
            pltpu.SemaphoreType.DMA((len(vch),)),
            pltpu.SemaphoreType.DMA(()),
            pltpu.SemaphoreType.DMA((B,)),
        ],
        compiler_params=pltpu.CompilerParams(
            vmem_limit_bytes=64 * 1024 * 1024,
        ),
    )(x2, k_cache, v_cache, wq, wo)
    return out.reshape(B, Sq, D)
```

```python
import functools

import jax
import jax.numpy as jnp
from jax import lax
import jax.experimental.pallas as pl
import jax.experimental.pallas.tpu as pltpu

_NB = 4
_NCH = 2


def _kernel(x_hbm, k_hbm, v_hbm, wq_hbm, wo_hbm, o_hbm,
            x_buf, k_buf, v_buf, wq_buf, wo_buf,
            acc_ref, q_ref, s_ref, p_ref, l_ref, oh_ref, ostage,
            sems, sems_last, sem_x, sem_o,
            *, B, Sq, H, Dh, rep, scale, vch):
    NB, NCH = _NB, _NCH
    HB = B // NCH
    PD = NB - 2
    LSLOT = (H - 1) % NB

    def rows(b):
        return slice(b * Sq, (b + 1) * Sq)

    def wq_copy(h, slot):
        off = pl.multiple_of(h * Dh, Dh)
        return pltpu.make_async_copy(
            wq_hbm.at[:, pl.ds(off, Dh)], wq_buf.at[slot], sems.at[0, slot])

    def wo_copy(h, slot):
        off = pl.multiple_of(h * Dh, Dh)
        return pltpu.make_async_copy(
            wo_hbm.at[pl.ds(off, Dh), :], wo_buf.at[slot], sems.at[1, slot])

    def k_copy(h, slot, c):
        return pltpu.make_async_copy(
            k_hbm.at[pl.ds(c * HB, HB), h // rep],
            k_buf.at[slot, pl.ds(c * HB, HB)], sems.at[2 + c, slot])

    def v_copy(h, slot, c):
        return pltpu.make_async_copy(
            v_hbm.at[pl.ds(c * HB, HB), h // rep],
            v_buf.at[slot, pl.ds(c * HB, HB)], sems.at[2 + NCH + c, slot])

    def v_last_copy(i):
        b0, b1 = vch[i]
        return pltpu.make_async_copy(
            v_hbm.at[pl.ds(b0, b1 - b0), (H - 1) // rep],
            v_buf.at[LSLOT, pl.ds(b0, b1 - b0)], sems_last.at[i])

    def out_copy(b):
        return pltpu.make_async_copy(
            ostage.at[rows(b), :], o_hbm.at[rows(b), :], sem_o.at[b])

    def start_head(h, slot):
        for c in range(NCH):
            k_copy(h, slot, c).start()
            v_copy(h, slot, c).start()
            if c == 0:
                wo_copy(h, slot).start()

    def start_last():
        for c in range(NCH):
            k_copy(H - 1, LSLOT, c).start()
        wo_copy(H - 1, LSLOT).start()
        for i in range(len(vch)):
            v_last_copy(i).start()

    x_copy = pltpu.make_async_copy(x_hbm, x_buf, sem_x)
    x_copy.start()
    wq_copy(0, 0).start()
    wq_copy(1, 1).start()
    for i in range(PD):
        start_head(i, i)
        wq_copy(i + 2, (i + 2) % NB).start()

    acc_ref[...] = jnp.zeros_like(acc_ref)
    s_ref[rows(B - 1), :] = jnp.zeros((Sq, s_ref.shape[1]), s_ref.dtype)
    p_ref[rows(B - 2), :] = jnp.zeros((Sq, p_ref.shape[1]), p_ref.dtype)
    l_ref[rows(B - 2), :] = jnp.ones((Sq, 1), l_ref.dtype)
    oh_ref[rows(B - 3), :] = jnp.zeros((Sq, Dh), oh_ref.dtype)
    x_copy.wait()
    wq_copy(0, 0).wait()
    q_ref[0] = jnp.dot(x_buf[...], wq_buf[0],
                       preferred_element_type=jnp.float32).astype(q_ref.dtype)

    def qproj(b, qs, wslot):
        q_ref[qs, rows(b), :] = jnp.dot(
            x_buf[rows(b), :], wq_buf[wslot],
            preferred_element_type=jnp.float32).astype(q_ref.dtype)

    def qk(b, qs, slot):
        s_ref[rows(b), :] = lax.dot_general(
            q_ref[qs, rows(b), :], k_buf[slot, b], (((1,), (1,)), ((), ())),
            preferred_element_type=jnp.float32)

    def softmax(b):
        s = s_ref[rows(b), :]
        m = jnp.max(s, axis=-1, keepdims=True)
        p = jnp.exp((s - m) * scale)
        l_ref[rows(b), :] = jnp.sum(p, axis=-1, keepdims=True)
        p_ref[rows(b), :] = p.astype(p_ref.dtype)

    def pv(b, slot, valid=None):
        vb = b if valid is None else jnp.where(valid, b, 0)
        o = jnp.dot(p_ref[rows(b), :], v_buf[slot, vb],
                    preferred_element_type=jnp.float32)
        o = o / l_ref[rows(b), :]
        if valid is not None:
            o = jnp.where(valid, o, 0.0)
        oh_ref[rows(b), :] = o.astype(oh_ref.dtype)

    def outp(b, slot, final=False):
        r = acc_ref[rows(b), :] + jnp.dot(
            oh_ref[rows(b), :], wo_buf[slot],
            preferred_element_type=jnp.float32)
        if final:
            ostage[rows(b), :] = r.astype(ostage.dtype)
            out_copy(b).start()
        else:
            acc_ref[rows(b), :] = r

    def body(h, carry):
        slot = h % NB
        pslot = jnp.maximum(h - 1, 0) % NB
        qs = h % 2
        has_prev = h > 0
        nxt = h + PD

        @pl.when(nxt < H - 1)
        def _():
            start_head(nxt, nxt % NB)

        @pl.when(nxt == H - 1)
        def _():
            start_last()

        @pl.when(nxt + 2 < H)
        def _():
            wq_copy(nxt + 2, (nxt + 2) % NB).start()

        wslot = (h + 1) % NB
        wq_copy(h + 1, wslot).wait()
        wo_copy(h, slot).wait()
        for t in range(B):
            if t % HB == 0:
                k_copy(h, slot, t // HB).wait()
                v_copy(h, slot, t // HB).wait()
            qk(t, qs, slot)
            softmax((t - 1) % B)
            if t >= 2:
                pv(t - 2, slot)
            else:
                pv(B + t - 2, pslot, has_prev)
            if t >= 3:
                outp(t - 3, slot)
            else:
                outp(B + t - 3, pslot)
            qproj(t, 1 - qs, wslot)
        return carry

    lax.fori_loop(0, H - 1, body, 0)

    qs = (H - 1) % 2
    pslot = (H - 2) % NB
    for t in range(B + 1):
        if t < B and t % HB == 0:
            k_copy(H - 1, LSLOT, t // HB).wait()
        if t < B:
            qk(t, qs, LSLOT)
        softmax((t - 1) % B)
        if t < 2:
            pv(B + t - 2, pslot)
        if t < 3:
            outp(B + t - 3, pslot)
    wo_copy(H - 1, LSLOT).wait()
    for i, (b0, b1) in enumerate(vch):
        v_last_copy(i).wait()
        for b in range(b0, b1):
            pv(b, LSLOT)
        for b in range(b0, b1):
            outp(b, LSLOT, final=True)
    for b in range(B):
        out_copy(b).wait()


@jax.jit
def pallas_standalone__gqa_block_cached__near_ridge_kernel(
    x: jax.Array,
    k_cache: jax.Array,
    v_cache: jax.Array,
    wq: jax.Array,
    wo: jax.Array,
):
    B, Sq, D = x.shape
    Hq, Dh = 32, 128
    Hkv, Sk = k_cache.shape[1], k_cache.shape[2]
    rep = Hq // Hkv
    M = B * Sq
    x2 = x.reshape(M, D)
    vch = ((0, B // 2), (B // 2, B - 1), (B - 1, B))

    kern = functools.partial(_kernel, B=B, Sq=Sq, H=Hq, Dh=Dh, rep=rep,
                             scale=float(Dh) ** -0.5, vch=vch)
    any_spec = pl.BlockSpec(memory_space=pl.ANY)
    out = pl.pallas_call(
        kern,
        in_specs=[any_spec] * 5,
        out_specs=any_spec,
        out_shape=jax.ShapeDtypeStruct((M, D), x.dtype),
        scratch_shapes=[
            pltpu.VMEM((M, D), x.dtype),
            pltpu.VMEM((_NB, B, Sk, Dh), k_cache.dtype),
            pltpu.VMEM((_NB, B, Sk, Dh), v_cache.dtype),
            pltpu.VMEM((_NB, D, Dh), wq.dtype),
            pltpu.VMEM((_NB, Dh, D), wo.dtype),
            pltpu.VMEM((M, D), jnp.float32),
            pltpu.VMEM((2, M, Dh), jnp.bfloat16),
            pltpu.VMEM((M, Sk), jnp.float32),
            pltpu.VMEM((M, Sk), jnp.bfloat16),
            pltpu.VMEM((M, 1), jnp.float32),
            pltpu.VMEM((M, Dh), jnp.bfloat16),
            pltpu.VMEM((M, D), x.dtype),
            pltpu.SemaphoreType.DMA((2 + 2 * _NCH, _NB)),
            pltpu.SemaphoreType.DMA((len(vch),)),
            pltpu.SemaphoreType.DMA(()),
            pltpu.SemaphoreType.DMA((B,)),
        ],
        compiler_params=pltpu.CompilerParams(
            vmem_limit_bytes=64 * 1024 * 1024,
        ),
    )(x2, k_cache, v_cache, wq, wo)
    return out.reshape(B, Sq, D)
```
